```python
import os as _os
_os.environ.setdefault("JAX_PLATFORMS", "cpu")
import jax
import jax.numpy as jnp

def _softmax(x, axis=-1):
    return jax.nn.softmax(x, axis=axis)
def _gelu(x):
    return jax.nn.gelu(x, approximate=True)
def _silu(x):
    return jax.nn.silu(x)
def _sigmoid(x):
    return jax.nn.sigmoid(x)
def _layernorm(x, axis=-1, eps=1e-5):
    m = jnp.mean(x, axis=axis, keepdims=True)
    v = jnp.var(x, axis=axis, keepdims=True)
    return (x - m) / jnp.sqrt(v + eps)
def _scatter_add(tgt, idx, src, axis=0):
    return tgt.at[idx].add(src)
def _segment_sum(src, seg, n):
    return jax.ops.segment_sum(src, seg, n)
class _Rng:
    def __init__(self, key):
        self._k = key
    def _next(self):
        self._k, sub = jax.random.split(self._k)
        return sub
    def normal(self, shape):
        return jax.random.normal(self._next(), shape, dtype=jnp.bfloat16)
    def randint(self, lo, hi, shape):
        return jax.random.randint(self._next(), shape, lo, hi, dtype=jnp.int32)
    def uniform(self, shape, lo=0.0, hi=1.0):
        return jax.random.uniform(self._next(), shape, jnp.bfloat16, lo, hi)
    def permutation(self, n):
        return jax.random.permutation(self._next(), n)


kernel_name = 'sequential_preLN__mha_block__dense_activation_mish__prompt'

def setup_inputs():
    _rng = _Rng(jax.random.key(int.from_bytes(__import__("os").urandom(4), "little")))
    _w = (lambda a: (lambda t: t.astype(jnp.bfloat16) if jnp.issubdtype(t.dtype, jnp.floating) else t)(jnp.asarray(a)))
    def _A_setup():
        B, S, D, H = 1, 2048, 576, 32
        return {
            "x": _w((lambda *s: _rng.normal(s) * 0.05)(B, S, D)),
            "wqkv": _w((lambda *s: _rng.normal(s) * 0.05)(D, 3 * D)),
            "wo": _w((lambda *s: _rng.normal(s) * 0.05)(D, D)),
        }
    _A_in = _A_setup()

    def _B_setup():
        B, S, D, F = 1, 2048, 576, 4608
        return {
            "x": _w((lambda *s: _rng.normal(s) * 0.05)(B, S, D)),
            "w1": _w((lambda *s: _rng.normal(s) * 1.6)(D, F) * (D ** -0.5)),
            "b1": _w((lambda *s: _rng.normal(s) * 0.05)(F)),
            "w2": _w((lambda *s: _rng.normal(s) * 0.05)(F, D) * (F ** -0.5)),
        }
    _B_in = _B_setup()

    return {
        "A_x": _A_in["x"],
        "A_wqkv": _A_in["wqkv"],
        "A_wo": _A_in["wo"],
        "B_x": _B_in["x"],
        "B_w1": _B_in["w1"],
        "B_b1": _B_in["b1"],
        "B_w2": _B_in["w2"],
    }

def reference(A_x, A_wqkv, A_wo, B_x, B_w1, B_b1, B_w2):
    def _A_ref(x, wqkv, wo):
        B, S, D = x.shape
        H = 32
        Dh = D // H
        qkv = (lambda x, *d: x.transpose(*d))((x @ wqkv).reshape(B, S, 3, H, Dh), 2, 0, 3, 1, 4)
        q, k, v = qkv[0], qkv[1], qkv[2]
        scores = jnp.einsum("bhqd,bhkd->bhqk", q, k) * (Dh ** -0.5)
        p = _softmax(scores, axis=-1)
        o = jnp.einsum("bhqk,bhkd->bhqd", p, v)
        return (lambda x, *d: x.transpose(*d))(o, 0, 2, 1, 3).reshape(B, S, D) @ wo

    def _B_ref(x, w1, b1, w2):
        h = jnp.einsum("bsd,df->bsf", x, w1) + b1
        sp = jnp.log1p(jnp.exp(-jnp.abs(h))) + jnp.where(h > 0, h, jnp.zeros_like(h))
        act = h * jnp.tanh(sp)
        return jnp.einsum("bsf,fd->bsd", act, w2)

    x = A_x
    h = x + _A_ref(_layernorm(x, axis=-1), A_wqkv, A_wo)
    h2 = h + _B_ref(_layernorm(h, axis=-1), B_w1, B_b1, B_w2)
    return h2
```

```python
import jax
import jax.numpy as jnp
import numpy as np
from jax import lax
import jax.experimental.pallas as pl
import jax.experimental.pallas.tpu as pltpu

S, D, H, DH, F = 2048, 576, 32, 18, 4608
G, HPG = 5, 7
VR = 24
LOG2E = 1.4426950408889634
F32, BF16 = jnp.float32, jnp.bfloat16
NN = (((1,), (0,)), ((), ()))
NT = (((1,), (1,)), ((), ()))
TN = (((0,), (0,)), ((), ()))

CFG = dict(bm1=512, bq=512, bk=128, bm3=512, fc=512, phases="123", flags=None)


def _ln(x):
    m = jnp.mean(x, axis=-1, keepdims=True)
    c = x - m
    v = jnp.mean(c * c, axis=-1, keepdims=True)
    return c * lax.rsqrt(v + 1e-5)


def _ln_t(x):
    m = jnp.mean(x, axis=0, keepdims=True)
    c = x - m
    v = jnp.mean(c * c, axis=0, keepdims=True)
    return c * lax.rsqrt(v + 1e-5)


def _mish(h):
    e = jnp.exp2(jnp.minimum(h, 20.0) * LOG2E)
    n = e * (e + 2.0)
    return h * (n / (n + 2.0))


def make(cfg):
    bm1, bq, bk, bm3, fc = cfg["bm1"], cfg["bq"], cfg["bk"], cfg["bm3"], cfg["fc"]
    phases = cfg["phases"]
    nq, nc = S // bq, S // bk

    def kern(xt_hbm, wqkv_hbm, wo_hbm, w1_hbm, b1_v, w2t_hbm, out_hbm,
             x_v, wqkv_v, wo_v, w1_v, w2_v, out_v,
             wk_s, wqt_s, wvt_s, wop_s, k_s, qt_s, vt_s, ot_s, s0, s1, m0, m1, sems):
        cp_x = pltpu.make_async_copy(xt_hbm, x_v, sems.at[0])
        cp_qkv = pltpu.make_async_copy(wqkv_hbm, wqkv_v, sems.at[1])
        cp_wo = pltpu.make_async_copy(wo_hbm, wo_v, sems.at[2])
        cp_w1 = pltpu.make_async_copy(w1_hbm, w1_v, sems.at[3])
        cp_w2 = pltpu.make_async_copy(w2t_hbm, w2_v, sems.at[5])
        cp_qkv.start(); cp_x.start()

        cp_qkv.wait()
        for g in range(G):
            wk_s[:, 128 * g:128 * (g + 1)] = wqkv_v[:, D + 126 * g:D + 126 * g + 128]
            wqt_s[128 * g:128 * (g + 1), :] = wqkv_v[:, 126 * g:126 * g + 128].T
        for t in range(0, D, 128):
            w = min(128, D - t)
            if w == 128:
                wvt_s[t:t + 128, :] = wqkv_v[:, 2 * D + t:2 * D + t + 128].T
            else:
                wvt_s[t:t + w, :] = wqkv_v[:, 3 * D - 128:3 * D].T[128 - w:, :]
        cp_x.wait()
        cp_wo.start(); cp_w1.start(); cp_w2.start()
        qscale = np.float32(DH ** -0.5 * LOG2E)
        if "1" in phases:
            for i in range(S // bm1):
                rows = slice(i * bm1, (i + 1) * bm1)
                ln = _ln_t(x_v[:, rows].astype(F32)).astype(BF16)
                kk = lax.dot_general(ln, wk_s[...], TN, preferred_element_type=F32).astype(BF16)
                for g in range(G):
                    k_s[g, rows, :] = kk[:, 128 * g:128 * (g + 1)]
                qt = lax.dot_general(wqt_s[...], ln, NN, preferred_element_type=F32)
                qt = (qt * qscale).astype(BF16)
                for g in range(G):
                    qt_s[g, :, rows] = qt[128 * g:128 * (g + 1), :]
                vt = lax.dot_general(wvt_s[...], ln, NN, preferred_element_type=F32)
                vt = vt.astype(BF16).astype(F32)
                row = lax.broadcasted_iota(jnp.int32, (VR, bm1), 0)
                for h in range(H):
                    lo = min(DH * h, D - VR)
                    sh = DH * h - lo
                    blk = vt[lo:lo + VR, :]
                    if sh:
                        blk = pltpu.roll(blk, VR - sh, 0)
                    vt_s[h, :, rows] = jnp.where(row < DH, blk, jnp.where(row == DH, 1.0, 0.0))

        n_it = H * nq

        def load_q(i):
            qb, h = i // H, i % H
            g = h // HPG
            j = h - g * HPG
            q = qt_s[g, :, pl.ds(pl.multiple_of(qb * bq, bq), bq)]
            qi = pltpu.bitcast(q, jnp.int32)
            r = lax.broadcasted_iota(jnp.int32, qi.shape, 0)
            msk = jnp.where((r >= j * (DH // 2)) & (r < j * (DH // 2) + DH // 2), -1, 0)
            return pltpu.bitcast(qi & msk, BF16), g

        def pass1(qm, g, c, s_scr, mp):
            k = k_s[g, c * bk:(c + 1) * bk, :]
            s = lax.dot_general(k, qm, NN, preferred_element_type=F32)
            s_scr[c * bk:(c + 1) * bk, :] = s
            pm = jnp.max(s.reshape(bk // 8, 8, bq), axis=0)
            return pm if mp is None else jnp.maximum(mp, pm)

        def pass2(m, h, c, s_scr, acc):
            s = s_scr[c * bk:(c + 1) * bk, :]
            p = jnp.exp2(s - m).astype(BF16)
            v = vt_s[h, :, c * bk:(c + 1) * bk]
            r = lax.dot_general(v, p, NN, preferred_element_type=F32)
            return r if acc is None else acc + r

        if "2" in phases:
            qm, g = load_q(0)
            mp = None
            for c in range(nc):
                mp = pass1(qm, g, c, s0, mp)
            m0[...] = jnp.broadcast_to(jnp.max(mp, axis=0, keepdims=True), (8, bq))

            def step(i, s_cur, m_cur, s_nxt, m_nxt):
                qm, g = load_q(jnp.minimum(i + 1, n_it - 1))
                qb, h = i // H, i % H
                m = m_cur[0:1, :]
                mp, acc = None, None
                for c in range(nc):
                    mp = pass1(qm, g, c, s_nxt, mp)
                    acc = pass2(m, h, c, s_cur, acc)
                m_nxt[...] = jnp.broadcast_to(jnp.max(mp, axis=0, keepdims=True), (8, bq))
                l = acc[DH:DH + 1, :]
                ot_s[h, :, pl.ds(pl.multiple_of(qb * bq, bq), bq)] = acc / l

            def body(j, _):
                pl.when(j >= 0)(lambda: step(2 * j, s0, m0, s1, m1))
                pl.when(j >= -1)(lambda: step(2 * j + 1, s1, m1, s0, m0))
                return 0

            lax.fori_loop(0, n_it // 2, body, 0)

        cp_wo.wait()
        zero = jnp.zeros((VR - DH, D), F32)
        wof = wo_v[...].astype(F32)
        pieces = []
        for h in range(H):
            pieces += [wof[DH * h:DH * (h + 1)], zero]
        wop = jnp.concatenate(pieces, axis=0)
        wop_s[...] = wop.T.astype(BF16)
        cp_w1.wait(); cp_w2.wait()
        out_cps = []
        for i in range(S // bm3):
            rows = slice(i * bm3, (i + 1) * bm3)
            if "3" in phases:
                ot = ot_s[:, :, rows].reshape(H * VR, bm3).astype(BF16)
                attn = lax.dot_general(wop_s[...], ot, NN, preferred_element_type=F32)
                hres = x_v[:, rows].astype(F32) + attn
                ln2 = _ln_t(hres).T.astype(BF16)
                acc = hres
                for c in range(F // fc):
                    cols = slice(c * fc, (c + 1) * fc)
                    h1 = lax.dot_general(ln2, w1_v[:, cols], NN, preferred_element_type=F32)
                    h1 = h1 + b1_v[cols].astype(F32)[None, :]
                    act = _mish(h1).astype(BF16)
                    acc = acc + lax.dot_general(w2_v[:, cols], act, NT, preferred_element_type=F32)
                out_v[:, rows] = acc.astype(BF16)
            else:
                out_v[:, rows] = x_v[:, rows]
            cp = pltpu.make_async_copy(out_v.at[:, rows], out_hbm.at[:, rows], sems.at[6 + i])
            cp.start()
            out_cps.append(cp)
        for cp in out_cps:
            cp.wait()

    hbm = pl.BlockSpec(memory_space=pltpu.HBM)
    scratch = [
        pltpu.VMEM((D, S), BF16), pltpu.VMEM((D, 3 * D), BF16), pltpu.VMEM((D, D), BF16),
        pltpu.VMEM((D, F), BF16), pltpu.VMEM((D, F), BF16), pltpu.VMEM((D, S), BF16),
        pltpu.VMEM((D, 128 * G), BF16), pltpu.VMEM((128 * G, D), BF16), pltpu.VMEM((D, D), BF16),
        pltpu.VMEM((D, H * VR), BF16),
        pltpu.VMEM((G, S, 128), BF16), pltpu.VMEM((G, 128, S), BF16), pltpu.VMEM((H, VR, S), F32),
        pltpu.VMEM((H, VR, S), F32),
        pltpu.VMEM((S, bq), F32), pltpu.VMEM((S, bq), F32), pltpu.VMEM((8, bq), F32), pltpu.VMEM((8, bq), F32),
        pltpu.SemaphoreType.DMA((6 + S // bm3,)),
    ]

    def fn(A_x, A_wqkv, A_wo, B_x, B_w1, B_b1, B_w2):
        out = pl.pallas_call(
            kern,
            out_shape=jax.ShapeDtypeStruct((D, S), BF16),
            in_specs=[hbm, hbm, hbm, hbm, pl.BlockSpec((F,), lambda: (0,)), hbm],
            out_specs=hbm,
            scratch_shapes=scratch,
            compiler_params=pltpu.CompilerParams(vmem_limit_bytes=110 * 1024 * 1024, flags=cfg["flags"]),
            name="fused_" + "_".join(str(v) for k, v in cfg.items() if k != "flags"),
        )(A_x.reshape(S, D).T, A_wqkv, A_wo, B_w1, B_b1, B_w2.T)
        return out.T.reshape(1, S, D)

    return jax.jit(fn)


_kernel = make(dict(CFG))


@jax.jit
def pallas_sequential_preLN__mha_block__dense_activation_mish__prompt_kernel(
    A_x: jax.Array,
    A_wqkv: jax.Array,
    A_wo: jax.Array,
    B_x: jax.Array,
    B_w1: jax.Array,
    B_b1: jax.Array,
    B_w2: jax.Array,
):
    return _kernel(A_x, A_wqkv, A_wo, B_x, B_w1, B_b1, B_w2)
```

```python
import jax
import jax.numpy as jnp
import numpy as np
from jax import lax
import jax.experimental.pallas as pl
import jax.experimental.pallas.tpu as pltpu

S, D, H, DH, F = 2048, 576, 32, 18, 4608
G, HPG = 5, 7
VR = 24
LOG2E = 1.4426950408889634
F32, BF16 = jnp.float32, jnp.bfloat16
NN = (((1,), (0,)), ((), ()))
NT = (((1,), (1,)), ((), ()))
TN = (((0,), (0,)), ((), ()))

CFG = dict(bm1=512, bq=128, bk=128, hps=16, bm3=512, fc=768, wsplit=2, ep0=0, epn=18, xsplit=512, ep00=8,
           scopes=0, flags=None)


def _dot(a, b, dims):
    return lax.dot_general(a, b, dims, preferred_element_type=F32)


def _ln_t(x):
    m = jnp.mean(x, axis=0, keepdims=True)
    c = x - m
    v = jnp.mean(c * c, axis=0, keepdims=True)
    return c * lax.rsqrt(v + 1e-5)


def _mish(h):
    e = jnp.exp2(jnp.minimum(h, 20.0) * LOG2E)
    n = e * (e + 2.0)
    return h * (n / (n + 2.0))


class _Scopes:
    def __init__(self, on):
        self.on, self.cur = on, None

    def go(self, name):
        if not self.on:
            return
        if self.cur is not None:
            self.cur.__exit__(None, None, None)
            self.cur = None
        if name is not None:
            self.cur = jax.named_scope(name)
            self.cur.__enter__()


def make(cfg):
    bm1, bq, bk, bm3, fc, hps = cfg["bm1"], cfg["bq"], cfg["bk"], cfg["bm3"], cfg["fc"], cfg["hps"]
    assert 2 * hps == H
    nq, nc, nb1 = S // bq, S // bk, S // bm1
    QR = 128 * (G - 1) + 80

    def kern(xt_hbm, wqkv_hbm, wo_hbm, w1_hbm, b1_hbm, w2t_hbm, out_hbm,
             x_v, wqkv_v, wo_v, w1_v, w2_v, out_v, ln_s,
             wk_s, wqt_s, wvt_s, wot_s, k_s, qt_s, vt_s, ot_s, sems, b1_v, *bufs):
        sb = [bufs[0:hps], bufs[hps:2 * hps]]
        mb = [bufs[2 * hps:3 * hps], bufs[3 * hps:4 * hps]]
        sc = _Scopes(cfg["scopes"])

        def copy(src, dst, i):
            return pltpu.make_async_copy(src, dst, sems.at[i])

        xs = cfg["xsplit"]
        cp_x = copy(xt_hbm.at[:, 0:xs], x_v.at[:, 0:xs], 0)
        cp_wk = copy(wqkv_hbm.at[:, 512:1280], wqkv_v.at[:, 512:1280], 1)
        cp_wo = copy(wo_hbm, wo_v, 2)
        cp_w1 = copy(w1_hbm, w1_v, 3)
        cp_wq = copy(wqkv_hbm.at[:, 0:512], wqkv_v.at[:, 0:512], 4)
        cp_w2 = copy(w2t_hbm, w2_v, 5)
        cp_wv = copy(wqkv_hbm.at[:, 1280:3 * D], wqkv_v.at[:, 1280:3 * D], 6)
        cp_xr = copy(xt_hbm.at[:, xs:S], x_v.at[:, xs:S], 7)
        cp_b1 = copy(b1_hbm, b1_v, 8)
        cp_wk.start(); cp_x.start()
        sc.go("s_p1a")

        qscale = np.float32(DH ** -0.5 * LOG2E)

        def ln_block(i):
            cols = slice(i * bm1, (i + 1) * bm1)
            ln_s[:, cols] = _ln_t(x_v[:, cols].astype(F32)).astype(BF16)

        def k_block(i):
            rows = slice(i * bm1, (i + 1) * bm1)
            kk = _dot(ln_s[:, rows], wk_s[...], TN).astype(BF16)
            for g in range(G):
                k_s[g, rows, :] = kk[:, 128 * g:128 * (g + 1)]

        def qv_block(i):
            rows = slice(i * bm1, (i + 1) * bm1)
            ln = ln_s[:, rows]
            qt = (_dot(wqt_s[0:QR, :], ln, NN) * qscale).astype(BF16)
            for g in range(G):
                r = min(128, QR - 128 * g)
                qt_s[g, 0:r, rows] = qt[128 * g:128 * g + r, :]
            vt = _dot(wvt_s[...], ln, NN).astype(BF16).astype(F32)
            row = lax.broadcasted_iota(jnp.int32, (VR, bm1), 0)
            for h in range(H):
                lo = min(DH * h, D - VR)
                sh = DH * h - lo
                blk = vt[lo:lo + VR, :]
                if sh:
                    blk = pltpu.roll(blk, VR - sh, 0)
                vt_s[h, :, rows] = jnp.where(row < DH, blk, jnp.where(row == DH, 1.0, 0.0))

        cp_wk.wait(); cp_x.wait()
        cp_xr.start()
        for g in range(G):
            wk_s[:, 128 * g:128 * (g + 1)] = wqkv_v[:, D + 126 * g:D + 126 * g + 128]
        ln_block(0)
        for i in range(nb1):
            if i == cfg["wsplit"]:
                cp_wq.wait(); cp_wv.wait()
                cp_wo.start(); cp_b1.start(); cp_w1.start(); cp_w2.start()
                for g in range(G):
                    wqt_s[128 * g:128 * (g + 1), :] = wqkv_v[:, 126 * g:126 * g + 128].T
                for t in range(0, D, 128):
                    w = min(128, D - t)
                    if w == 128:
                        wvt_s[t:t + 128, :] = wqkv_v[:, 2 * D + t:2 * D + t + 128].T
                    else:
                        wvt_s[t:t + w, :] = wqkv_v[:, 3 * D - 128:3 * D].T[128 - w:, :]
            if (i + 1) * bm1 == xs:
                k_block(i)
                cp_xr.wait()
                cp_wq.start(); cp_wv.start()
                ln_block(i + 1)
                continue
            if i + 1 < nb1:
                ln_block(i + 1)
            k_block(i)
        sc.go("s_p1b")
        for i in range(nb1):
            qv_block(i)

        def qcols(qb):
            return pl.ds(pl.multiple_of(qb * bq, bq), bq)

        def load_q(qb, h):
            g, j = divmod(h, HPG)
            lo, hi = DH * j // 16 * 16, -(-DH * (j + 1) // 16) * 16
            qi = pltpu.bitcast(qt_s[g, lo:hi, qcols(qb)], jnp.int32)
            r = lax.broadcasted_iota(jnp.int32, qi.shape, 0) + lo // 2
            own = (r >= j * (DH // 2)) & (r < (j + 1) * (DH // 2))
            q = pltpu.bitcast(jnp.where(own, qi, 0), BF16)
            parts = [jnp.zeros((lo, bq), BF16)] * (lo > 0) + [q] + [jnp.zeros((128 - hi, bq), BF16)] * (hi < 128)
            return jnp.concatenate(parts, axis=0)

        def pass1(qm, h, c, s_scr, mp):
            s = _dot(k_s[h // HPG, c * bk:(c + 1) * bk, :], qm, NN)
            s_scr[c * bk:(c + 1) * bk, :] = s
            pm = jnp.max(s.reshape(bk // 8, 8, bq), axis=0)
            return pm if mp is None else jnp.maximum(mp, pm)

        def pass2(m, h, c, s_scr, acc):
            p = jnp.exp2(s_scr[c * bk:(c + 1) * bk, :] - m).astype(BF16)
            r = _dot(vt_s[h, :, c * bk:(c + 1) * bk], p, NN)
            return r if acc is None else acc + r

        def step(qb2, half2, qb1, half1):
            do2, do1 = qb2 is not None, qb1 is not None
            qs = [load_q(qb1, half1 * hps + u) for u in range(hps)] if do1 else None
            ms = [mb[half2][u][0:1, :] for u in range(hps)] if do2 else None
            mp, acc = [None] * hps, [None] * hps
            for c in range(nc):
                for u in range(hps):
                    if do2:
                        acc[u] = pass2(ms[u], half2 * hps + u, c, sb[half2][u], acc[u])
                    if do1:
                        mp[u] = pass1(qs[u], half1 * hps + u, c, sb[half1][u], mp[u])
                    yield
            if do1:
                for u in range(hps):
                    mb[half1][u][...] = jnp.broadcast_to(jnp.max(mp[u], axis=0, keepdims=True), (8, bq))
            if do2:
                o = jnp.concatenate([(a / a[DH:DH + 1, :])[0:DH, :] for a in acc], axis=0)
                ot_s[half2 * hps * DH:(half2 + 1) * hps * DH, qcols(qb2)] = o
            yield

        def run(gen):
            for _ in gen:
                pass

        sc.go("s_prologue")
        run(step(None, None, 0, 0))
        sc.go("s_loop")

        def body(j, _):
            pl.when(j >= 0)(lambda: run(step(j, 0, j, 1)))
            pl.when(j < nq - 1)(lambda: run(step(j, 1, j + 1, 0)))
            return 0

        lax.fori_loop(0, nq, body, 0)
        sc.go("s_p3")
        ep = step(nq - 1, 1, None, None)
        n_units = nc * hps + 1

        def drain(n):
            for _ in range(n):
                next(ep, None)

        cp_wo.wait(); cp_b1.wait(); cp_w1.wait(); cp_w2.wait()
        drain(cfg["ep00"])
        wot_s[...] = wo_v[...].astype(F32).T.astype(BF16)
        out_cps = []
        nb3 = S // bm3
        for i in range(nb3):
            rows = slice(i * bm3, (i + 1) * bm3)
            if i == nb3 - 1:
                drain(n_units)
            attn = _dot(wot_s[...], ot_s[:, rows].astype(BF16), NN)
            hres = x_v[:, rows].astype(F32) + attn
            ln2 = _ln_t(hres).T.astype(BF16)
            drain(cfg["ep0"])
            acc = hres
            for c in range(F // fc):
                cols = slice(c * fc, (c + 1) * fc)
                h1 = _dot(ln2, w1_v[:, cols], NN) + b1_v[cols].astype(F32)[None, :]
                act = _mish(h1).astype(BF16)
                acc = acc + _dot(w2_v[:, cols], act, NT)
                drain(-(-n_units // cfg["epn"]))
            out_v[:, rows] = acc.astype(BF16)
            cp = copy(out_v.at[:, rows], out_hbm.at[:, rows], 9 + i)
            cp.start()
            out_cps.append(cp)
        sc.go("s_outwait")
        for cp in out_cps:
            cp.wait()
        sc.go(None)

    hbm = pl.BlockSpec(memory_space=pltpu.HBM)
    scratch = [
        pltpu.VMEM((D, S), BF16), pltpu.VMEM((D, 3 * D), BF16), pltpu.VMEM((D, D), BF16),
        pltpu.VMEM((D, F), BF16), pltpu.VMEM((D, F), BF16), pltpu.VMEM((D, S), BF16), pltpu.VMEM((D, S), BF16),
        pltpu.VMEM((D, 128 * G), BF16), pltpu.VMEM((128 * G, D), BF16), pltpu.VMEM((D, D), BF16),
        pltpu.VMEM((D, D), BF16),
        pltpu.VMEM((G, S, 128), BF16), pltpu.VMEM((G, 128, S), BF16), pltpu.VMEM((H, VR, S), F32),
        pltpu.VMEM((D, S), F32),
        pltpu.SemaphoreType.DMA((9 + S // bm3,)), pltpu.VMEM((F,), BF16),
    ] + [pltpu.VMEM((S, bq), F32)] * (2 * hps) + [pltpu.VMEM((8, bq), F32)] * (2 * hps)

    def fn(A_x, A_wqkv, A_wo, B_x, B_w1, B_b1, B_w2):
        out = pl.pallas_call(
            kern,
            out_shape=jax.ShapeDtypeStruct((D, S), BF16),
            in_specs=[hbm] * 6,
            out_specs=hbm,
            scratch_shapes=scratch,
            compiler_params=pltpu.CompilerParams(vmem_limit_bytes=120 * 1024 * 1024, flags=cfg["flags"]),
            name="fused_" + "_".join(str(v) for k, v in cfg.items() if k != "flags"),
        )(A_x.reshape(S, D).T, A_wqkv, A_wo, B_w1, B_b1, B_w2.T)
        return out.T.reshape(1, S, D)

    return jax.jit(fn)


_kernel = make(dict(CFG))


@jax.jit
def pallas_sequential_preLN__mha_block__dense_activation_mish__prompt_kernel(
    A_x: jax.Array,
    A_wqkv: jax.Array,
    A_wo: jax.Array,
    B_x: jax.Array,
    B_w1: jax.Array,
    B_b1: jax.Array,
    B_w2: jax.Array,
):
    return _kernel(A_x, A_wqkv, A_wo, B_x, B_w1, B_b1, B_w2)
```

```python
import jax
import jax.numpy as jnp
import numpy as np
from jax import lax
import jax.experimental.pallas as pl
import jax.experimental.pallas.tpu as pltpu

S, D, H, DH, F = 2048, 576, 32, 18, 4608
G, HPG = 5, 7
QR = 592
KLR = 80
VR = 24
LOG2E = 1.4426950408889634
F32, BF16 = jnp.float32, jnp.bfloat16
NN = (((1,), (0,)), ((), ()))
NT = (((1,), (1,)), ((), ()))
TN = (((0,), (0,)), ((), ()))

CFG = dict(bm1=256, xs=512, ws=4, bq=128, bk=128, bm3=512, fc=768, ep00=8, epn=18, tail=1, scopes=0, flags=None)


def _dot(a, b, dims):
    return lax.dot_general(a, b, dims, preferred_element_type=F32)


def _ln_t(x):
    m = jnp.mean(x, axis=0, keepdims=True)
    c = x - m
    v = jnp.mean(c * c, axis=0, keepdims=True)
    return c * lax.rsqrt(v + 1e-5)


def _mish(h):
    e = jnp.exp2(jnp.minimum(h, 20.0) * LOG2E)
    n = e * (e + 2.0)
    return h * (n / (n + 2.0))


class _Scopes:
    def __init__(self, on):
        self.on, self.cur = on, None

    def go(self, name):
        if not self.on:
            return
        if self.cur is not None:
            self.cur.__exit__(None, None, None)
            self.cur = None
        if name is not None:
            self.cur = jax.named_scope(name)
            self.cur.__enter__()


def make(cfg):
    bm1, xs, bq, bk, bm3, fc = cfg["bm1"], cfg["xs"], cfg["bq"], cfg["bk"], cfg["bm3"], cfg["fc"]
    hps = H // 2
    nq, nc, nb1, nb3 = S // bq, S // bk, S // bm1, S // bm3

    def kern(xt_hbm, wqkv_hbm, wo_hbm, w1_hbm, b1_hbm, w2t_hbm, out_hbm,
             x_v, wqkv_v, wo_v, w1_v, w2_v, out_v, ln_s,
             wk_s, wkl_s, wqt_s, wvt_s, wot_s, k_s, qt_s, vt_s, ot_s, sems, b1_v, *bufs):
        sb = [bufs[0:hps], bufs[hps:2 * hps]]
        mb = [bufs[2 * hps:3 * hps], bufs[3 * hps:4 * hps]]
        sc = _Scopes(cfg["scopes"])

        def copy(src, dst, i):
            return pltpu.make_async_copy(src, dst, sems.at[i])

        cp_x = copy(xt_hbm.at[:, 0:xs], x_v.at[:, 0:xs], 0)
        cp_wk = copy(wqkv_hbm.at[:, 512:2 * D], wqkv_v.at[:, 512:2 * D], 1)
        cp_wo = copy(wo_hbm, wo_v, 2)
        cp_w1 = copy(w1_hbm, w1_v, 3)
        cp_wq = copy(wqkv_hbm.at[:, 0:512], wqkv_v.at[:, 0:512], 4)
        cp_w2 = copy(w2t_hbm, w2_v, 5)
        cp_wv = copy(wqkv_hbm.at[:, 2 * D:3 * D], wqkv_v.at[:, 2 * D:3 * D], 6)
        cp_xr = copy(xt_hbm.at[:, xs:S], x_v.at[:, xs:S], 7)
        cp_b1 = copy(b1_hbm, b1_v, 8)

        qscale = np.float32(DH ** -0.5 * LOG2E)

        def ln_block(i):
            cols = slice(i * bm1, (i + 1) * bm1)
            ln_s[:, cols] = _ln_t(x_v[:, cols].astype(F32)).astype(BF16)

        def k_block(i):
            rows = slice(i * bm1, (i + 1) * bm1)
            ln = ln_s[:, rows]
            kk = _dot(ln, wk_s[...], TN).astype(BF16)
            for g in range(G - 1):
                k_s[g, rows, :] = kk[:, 128 * g:128 * (g + 1)]
            klt = _dot(wkl_s[...], ln, NN)
            klt = jnp.concatenate([klt, jnp.zeros((128 - KLR, bm1), F32)], axis=0)
            k_s[G - 1, rows, :] = klt.T.astype(BF16)

        def qv_block(i):
            rows = slice(i * bm1, (i + 1) * bm1)
            ln = ln_s[:, rows]
            qt = (_dot(wqt_s[0:QR, :], ln, NN) * qscale).astype(BF16)
            for g in range(G):
                r = min(128, QR - 128 * g)
                qt_s[g, 0:r, rows] = qt[128 * g:128 * g + r, :]
            vt = _dot(wvt_s[...], ln, NN).astype(BF16).astype(F32)
            row = lax.broadcasted_iota(jnp.int32, (VR, bm1), 0)
            for h in range(H):
                lo = min(DH * h, D - VR)
                sh = DH * h - lo
                blk = vt[lo:lo + VR, :]
                if sh:
                    blk = pltpu.roll(blk, VR - sh, 0)
                vt_s[h, :, rows] = jnp.where(row < DH, blk, jnp.where(row == DH, 1.0, 0.0))

        cp_wk.start(); cp_x.start()
        sc.go("s_w1")
        cp_wk.wait(); cp_x.wait()
        sc.go("s_p1a")
        cp_xr.start()
        for g in range(G - 1):
            wk_s[:, 128 * g:128 * (g + 1)] = wqkv_v[:, D + 126 * g:D + 126 * g + 128]
        wkl_s[...] = jnp.concatenate(
            [wqkv_v[:, 2 * D - 128:2 * D].astype(F32).T[56:, :], jnp.zeros((KLR - 72, D), F32)], axis=0).astype(BF16)
        ln_block(0)
        for i in range(nb1):
            if i == cfg["ws"]:
                cp_wq.wait(); cp_wv.wait()
                cp_wo.start(); cp_b1.start(); cp_w1.start(); cp_w2.start()
                for g in range(G):
                    wqt_s[128 * g:128 * (g + 1), :] = wqkv_v[:, 126 * g:126 * g + 128].T
                for t in range(0, D, 128):
                    w = min(128, D - t)
                    if w == 128:
                        wvt_s[t:t + 128, :] = wqkv_v[:, 2 * D + t:2 * D + t + 128].T
                    else:
                        wvt_s[t:t + w, :] = wqkv_v[:, 3 * D - 128:3 * D].T[128 - w:, :]
            k_block(i)
            if (i + 1) * bm1 == xs:
                cp_xr.wait()
                cp_wq.start(); cp_wv.start()
            if i + 1 < nb1:
                ln_block(i + 1)
        sc.go("s_p1b")
        for i in range(nb1):
            qv_block(i)

        def qcols(qb):
            return pl.ds(pl.multiple_of(qb * bq, bq), bq)

        def load_q(qb, h):
            g, j = divmod(h, HPG)
            lo, hi = DH * j // 16 * 16, -(-DH * (j + 1) // 16) * 16
            qi = pltpu.bitcast(qt_s[g, lo:hi, qcols(qb)], jnp.int32)
            r = lax.broadcasted_iota(jnp.int32, qi.shape, 0) + lo // 2
            own = (r >= j * (DH // 2)) & (r < (j + 1) * (DH // 2))
            q = pltpu.bitcast(jnp.where(own, qi, 0), BF16)
            parts = [jnp.zeros((lo, bq), BF16)] * (lo > 0) + [q] + [jnp.zeros((128 - hi, bq), BF16)] * (hi < 128)
            return jnp.concatenate(parts, axis=0)

        def pass1(qm, h, c, s_scr, mp):
            s = _dot(k_s[h // HPG, c * bk:(c + 1) * bk, :], qm, NN)
            s_scr[c * bk:(c + 1) * bk, :] = s
            pm = jnp.max(s.reshape(bk // 8, 8, bq), axis=0)
            return pm if mp is None else jnp.maximum(mp, pm)

        def pass2(m, h, c, s_scr, acc):
            p = jnp.exp2(s_scr[c * bk:(c + 1) * bk, :] - m).astype(BF16)
            r = _dot(vt_s[h, :, c * bk:(c + 1) * bk], p, NN)
            return r if acc is None else acc + r

        def step(qb2, half2, qb1, half1):
            do2, do1 = qb2 is not None, qb1 is not None
            outs = []
            for u in range(hps):
                h1, h2 = (half1 * hps + u if do1 else None), (half2 * hps + u if do2 else None)
                qm = load_q(qb1, h1) if do1 else None
                m = mb[half2][u][0:1, :] if do2 else None
                mp = acc = None
                for c in range(nc):
                    if do1:
                        mp = pass1(qm, h1, c, sb[half1][u], mp)
                    if do2:
                        acc = pass2(m, h2, c, sb[half2][u], acc)
                    yield
                if do1:
                    mb[half1][u][...] = jnp.broadcast_to(jnp.max(mp, axis=0, keepdims=True), (8, bq))
                if do2:
                    outs.append((acc / acc[DH:DH + 1, :])[0:DH, :])
                    if len(outs) == 4:
                        ot_s[(h2 - 3) * DH:(h2 + 1) * DH, qcols(qb2)] = jnp.concatenate(outs, axis=0)
                        outs = []

        def run(gen):
            for _ in gen:
                pass

        def body(j, carry):
            run(step(j, 0, j, 1))
            run(step(j, 1, j + 1, 0))
            return carry

        sc.go("s_prologue")
        run(step(None, None, 0, 0))
        sc.go("s_loop")
        lax.fori_loop(0, nq - 1, body, 0)
        run(step(nq - 1, 0, nq - 1, 1))
        sc.go("s_p3")
        ep = step(nq - 1, 1, None, None)
        n_units = nc * hps + 1

        def drain(n):
            for _ in range(n):
                next(ep, None)

        cp_wo.wait(); cp_b1.wait(); cp_w1.wait(); cp_w2.wait()
        drain(cfg["ep00"])
        wot_s[...] = wo_v[...].astype(F32).T.astype(BF16)
        out_cps = []

        def store_out(lo, hi, val):
            out_v[:, lo:hi] = val.astype(BF16)
            cp = copy(out_v.at[:, lo:hi], out_hbm.at[:, lo:hi], 9 + len(out_cps))
            cp.start()
            out_cps.append(cp)

        for i in range(nb3):
            lo, hi = i * bm3, (i + 1) * bm3
            last = i == nb3 - 1
            if last:
                drain(n_units)
            attn = _dot(wot_s[...], ot_s[:, lo:hi].astype(BF16), NN)
            hres = x_v[:, lo:hi].astype(F32) + attn
            ln2 = _ln_t(hres).T.astype(BF16)
            acc = hres
            for c in range(F // fc):
                cols = slice(c * fc, (c + 1) * fc)
                h1 = _dot(ln2, w1_v[:, cols], NN) + b1_v[cols].astype(F32)[None, :]
                act = _mish(h1).astype(BF16)
                if last and cfg["tail"] and c == F // fc - 1:
                    hb = bm3 // 2
                    for t in (0, hb):
                        store_out(lo + t, lo + t + hb, acc[:, t:t + hb] + _dot(w2_v[:, cols], act[t:t + hb, :], NT))
                else:
                    acc = acc + _dot(w2_v[:, cols], act, NT)
                drain(-(-n_units // cfg["epn"]))
            if not (last and cfg["tail"]):
                store_out(lo, hi, acc)
        sc.go("s_outwait")
        for cp in out_cps:
            cp.wait()
        sc.go(None)

    hbm = pl.BlockSpec(memory_space=pltpu.HBM)
    scratch = [
        pltpu.VMEM((D, S), BF16), pltpu.VMEM((D, 3 * D), BF16), pltpu.VMEM((D, D), BF16),
        pltpu.VMEM((D, F), BF16), pltpu.VMEM((D, F), BF16), pltpu.VMEM((D, S), BF16), pltpu.VMEM((D, S), BF16),
        pltpu.VMEM((D, 512), BF16), pltpu.VMEM((KLR, D), BF16), pltpu.VMEM((128 * G, D), BF16),
        pltpu.VMEM((D, D), BF16), pltpu.VMEM((D, D), BF16),
        pltpu.VMEM((G, S, 128), BF16), pltpu.VMEM((G, 128, S), BF16), pltpu.VMEM((H, VR, S), F32),
        pltpu.VMEM((D, S), F32),
        pltpu.SemaphoreType.DMA((10 + nb3,)), pltpu.VMEM((F,), BF16),
    ] + [pltpu.VMEM((S, bq), F32)] * (2 * hps) + [pltpu.VMEM((8, bq), F32)] * (2 * hps)

    def fn(A_x, A_wqkv, A_wo, B_x, B_w1, B_b1, B_w2):
        out = pl.pallas_call(
            kern,
            out_shape=jax.ShapeDtypeStruct((D, S), BF16),
            in_specs=[hbm] * 6,
            out_specs=hbm,
            scratch_shapes=scratch,
            compiler_params=pltpu.CompilerParams(vmem_limit_bytes=120 * 1024 * 1024, flags=cfg["flags"]),
            name="fused_" + "_".join(str(v) for k, v in cfg.items() if k != "flags"),
        )(A_x.reshape(S, D).T, A_wqkv, A_wo, B_w1, B_b1, B_w2.T)
        return out.T.reshape(1, S, D)

    return jax.jit(fn)


_kernel = make(dict(CFG))


@jax.jit
def pallas_sequential_preLN__mha_block__dense_activation_mish__prompt_kernel(
    A_x: jax.Array,
    A_wqkv: jax.Array,
    A_wo: jax.Array,
    B_x: jax.Array,
    B_w1: jax.Array,
    B_b1: jax.Array,
    B_w2: jax.Array,
):
    return _kernel(A_x, A_wqkv, A_wo, B_x, B_w1, B_b1, B_w2)
```

```python
import jax
import jax.numpy as jnp
import numpy as np
from jax import lax
import jax.experimental.pallas as pl
import jax.experimental.pallas.tpu as pltpu

S, D, H, DH, F = 2048, 576, 32, 18, 4608
G, HPG = 5, 7
QR = 592
KLR = 80
VR = 24
BM1 = 256
XS = 768
BQ, BK = 128, 128
HPS = H // 2
BM3, FC = 512, 768
NQ, NC, NB1, NB3 = S // BQ, S // BK, S // BM1, S // BM3
LOG2E = 1.4426950408889634
F32, BF16 = jnp.float32, jnp.bfloat16
NN = (((1,), (0,)), ((), ()))
NT = (((1,), (1,)), ((), ()))
TN = (((0,), (0,)), ((), ()))


def _dot(a, b, dims):
    return lax.dot_general(a, b, dims, preferred_element_type=F32)


def _ln_t(x):
    m = jnp.mean(x, axis=0, keepdims=True)
    c = x - m
    v = jnp.mean(c * c, axis=0, keepdims=True)
    return c * lax.rsqrt(v + 1e-5)


def _mish(h):
    e = jnp.exp2(jnp.minimum(h, 20.0) * LOG2E)
    n = e * (e + 2.0)
    return h * (n / (n + 2.0))


def _kernel(xt_hbm, wqkv_hbm, wo_hbm, w1_hbm, b1_hbm, w2t_hbm, out_hbm,
            x_v, wqkv_v, wo_v, w1_v, w2_v, out_v, ln_s,
            wk_s, wkl_s, wqt_s, wvt_s, wot_s, k_s, qt_s, vt_s, ot_s, sems, b1_v, *bufs):
    sb = [bufs[0:HPS], bufs[HPS:2 * HPS]]
    mb = [bufs[2 * HPS:3 * HPS], bufs[3 * HPS:4 * HPS]]

    def copy(src, dst, i):
        return pltpu.make_async_copy(src, dst, sems.at[i])

    cp_x = copy(xt_hbm.at[:, 0:XS], x_v.at[:, 0:XS], 0)
    cp_wk = copy(wqkv_hbm.at[:, 512:2 * D], wqkv_v.at[:, 512:2 * D], 1)
    cp_wo = copy(wo_hbm, wo_v, 2)
    cp_w1 = copy(w1_hbm, w1_v, 3)
    cp_wq = copy(wqkv_hbm.at[:, 0:512], wqkv_v.at[:, 0:512], 4)
    cp_w2 = copy(w2t_hbm, w2_v, 5)
    cp_wv = copy(wqkv_hbm.at[:, 2 * D:3 * D], wqkv_v.at[:, 2 * D:3 * D], 6)
    cp_xr = copy(xt_hbm.at[:, XS:S], x_v.at[:, XS:S], 7)
    cp_b1 = copy(b1_hbm, b1_v, 8)

    qscale = np.float32(DH ** -0.5 * LOG2E)

    def ln_block(i):
        cols = slice(i * BM1, (i + 1) * BM1)
        ln_s[:, cols] = _ln_t(x_v[:, cols].astype(F32)).astype(BF16)

    def k_block(i):
        rows = slice(i * BM1, (i + 1) * BM1)
        ln = ln_s[:, rows]
        klt = _dot(wkl_s[...], ln, NN)
        klt = jnp.concatenate([klt, jnp.zeros((128 - KLR, BM1), F32)], axis=0)
        k_s[G - 1, rows, :] = klt.T.astype(BF16)
        kk = _dot(ln, wk_s[...], TN).astype(BF16)
        for g in range(G - 1):
            k_s[g, rows, :] = kk[:, 128 * g:128 * (g + 1)]

    def qv_block(i):
        rows = slice(i * BM1, (i + 1) * BM1)
        ln = ln_s[:, rows]
        qt = (_dot(wqt_s[0:QR, :], ln, NN) * qscale).astype(BF16)
        for g in range(G):
            r = min(128, QR - 128 * g)
            qt_s[g, 0:r, rows] = qt[128 * g:128 * g + r, :]
        vt = _dot(wvt_s[...], ln, NN).astype(BF16).astype(F32)
        row = lax.broadcasted_iota(jnp.int32, (VR, BM1), 0)
        for h in range(H):
            lo = min(DH * h, D - VR)
            sh = DH * h - lo
            blk = vt[lo:lo + VR, :]
            if sh:
                blk = pltpu.roll(blk, VR - sh, 0)
            vt_s[h, :, rows] = jnp.where(row < DH, blk, jnp.where(row == DH, 1.0, 0.0))

    cp_wk.start(); cp_x.start()
    cp_wk.wait()
    for g in range(G - 1):
        wk_s[:, 128 * g:128 * (g + 1)] = wqkv_v[:, D + 126 * g:D + 126 * g + 128]
    wkl_s[...] = jnp.concatenate(
        [wqkv_v[:, 2 * D - 128:2 * D].astype(F32).T[56:, :], jnp.zeros((KLR - 72, D), F32)], axis=0).astype(BF16)
    cp_x.wait()
    cp_xr.start()
    nx0 = XS // BM1
    ln_block(0)
    for i in range(NB1):
        if i == nx0 - 1:
            cp_xr.wait()
            cp_wq.start(); cp_wv.start()
        if i == nx0 + 2:
            cp_wq.wait(); cp_wv.wait()
            cp_wo.start(); cp_b1.start(); cp_w1.start(); cp_w2.start()
        k_block(i)
        if i == nx0 + 2:
            for g in range(G):
                wqt_s[128 * g:128 * (g + 1), :] = wqkv_v[:, 126 * g:126 * g + 128].T
            for t in range(0, D - 128, 128):
                wvt_s[t:t + 128, :] = wqkv_v[:, 2 * D + t:2 * D + t + 128].T
            wvt_s[D - 64:D, :] = wqkv_v[:, 3 * D - 128:3 * D].T[64:, :]
        if i + 1 < NB1:
            ln_block(i + 1)
    for i in range(NB1):
        qv_block(i)

    def qcols(qb):
        return pl.ds(pl.multiple_of(qb * BQ, BQ), BQ)

    def load_q(qb, h):
        g, j = divmod(h, HPG)
        lo, hi = DH * j // 16 * 16, -(-DH * (j + 1) // 16) * 16
        qi = pltpu.bitcast(qt_s[g, lo:hi, qcols(qb)], jnp.int32)
        r = lax.broadcasted_iota(jnp.int32, qi.shape, 0) + lo // 2
        own = (r >= j * (DH // 2)) & (r < (j + 1) * (DH // 2))
        q = pltpu.bitcast(jnp.where(own, qi, 0), BF16)
        parts = [jnp.zeros((lo, BQ), BF16)] * (lo > 0) + [q] + [jnp.zeros((128 - hi, BQ), BF16)] * (hi < 128)
        return jnp.concatenate(parts, axis=0)

    def scores(qm, h, c, s_scr, mp):
        s = _dot(k_s[h // HPG, c * BK:(c + 1) * BK, :], qm, NN)
        s_scr[c * BK:(c + 1) * BK, :] = s
        pm = jnp.max(s.reshape(BK // 8, 8, BQ), axis=0)
        return pm if mp is None else jnp.maximum(mp, pm)

    def softmax_pv(m, h, c, s_scr, acc):
        p = jnp.exp2(s_scr[c * BK:(c + 1) * BK, :] - m).astype(BF16)
        r = _dot(vt_s[h, :, c * BK:(c + 1) * BK], p, NN)
        return r if acc is None else acc + r

    def step(qb2, half2, qb1, half1):
        do2, do1 = qb2 is not None, qb1 is not None
        outs = []
        for u in range(HPS):
            h1, h2 = (half1 * HPS + u if do1 else None), (half2 * HPS + u if do2 else None)
            qm = load_q(qb1, h1) if do1 else None
            m = mb[half2][u][0:1, :] if do2 else None
            mp = acc = None
            for c in range(NC):
                if do1:
                    mp = scores(qm, h1, c, sb[half1][u], mp)
                if do2:
                    acc = softmax_pv(m, h2, c, sb[half2][u], acc)
                yield
            if do1:
                mb[half1][u][...] = jnp.broadcast_to(jnp.max(mp, axis=0, keepdims=True), (8, BQ))
            if do2:
                outs.append((acc / acc[DH:DH + 1, :])[0:DH, :])
                if len(outs) == 4:
                    ot_s[(h2 - 3) * DH:(h2 + 1) * DH, qcols(qb2)] = jnp.concatenate(outs, axis=0)
                    outs = []

    def run(gen):
        for _ in gen:
            pass

    def body(j, carry):
        run(step(j, 0, j, 1))
        run(step(j, 1, j + 1, 0))
        return carry

    run(step(None, None, 0, 0))
    lax.fori_loop(0, NQ - 1, body, 0)
    run(step(NQ - 1, 0, NQ - 1, 1))
    tail = step(NQ - 1, 1, None, None)
    n_units = NC * HPS + 1

    def drain(n):
        for _ in range(n):
            next(tail, None)

    cp_wo.wait(); cp_b1.wait(); cp_w1.wait(); cp_w2.wait()
    drain(8)
    wot_s[...] = wo_v[...].astype(F32).T.astype(BF16)
    out_cps = []

    def store_out(lo, hi, val):
        out_v[:, lo:hi] = val.astype(BF16)
        cp = copy(out_v.at[:, lo:hi], out_hbm.at[:, lo:hi], 9 + len(out_cps))
        cp.start()
        out_cps.append(cp)

    for i in range(NB3):
        lo, hi = i * BM3, (i + 1) * BM3
        last = i == NB3 - 1
        if last:
            drain(n_units)
        attn = _dot(wot_s[...], ot_s[:, lo:hi].astype(BF16), NN)
        hres = x_v[:, lo:hi].astype(F32) + attn
        ln2 = _ln_t(hres).T.astype(BF16)
        acc = hres
        for c in range(F // FC):
            cols = slice(c * FC, (c + 1) * FC)
            h1 = _dot(ln2, w1_v[:, cols], NN) + b1_v[cols].astype(F32)[None, :]
            act = _mish(h1).astype(BF16)
            if last and c == F // FC - 1:
                hb = BM3 // 2
                for t in (0, hb):
                    store_out(lo + t, lo + t + hb, acc[:, t:t + hb] + _dot(w2_v[:, cols], act[t:t + hb, :], NT))
            else:
                acc = acc + _dot(w2_v[:, cols], act, NT)
            drain(-(-n_units // 18))
        if not last:
            store_out(lo, hi, acc)
    for cp in out_cps:
        cp.wait()


@jax.jit
def pallas_sequential_preLN__mha_block__dense_activation_mish__prompt_kernel(
    A_x: jax.Array,
    A_wqkv: jax.Array,
    A_wo: jax.Array,
    B_x: jax.Array,
    B_w1: jax.Array,
    B_b1: jax.Array,
    B_w2: jax.Array,
):
    del B_x
    hbm = pl.BlockSpec(memory_space=pltpu.HBM)
    vmem = pltpu.VMEM
    scratch = [
        vmem((D, S), BF16), vmem((D, 3 * D), BF16), vmem((D, D), BF16),
        vmem((D, F), BF16), vmem((D, F), BF16),
        vmem((D, S), BF16), vmem((D, S), BF16),
        vmem((D, 512), BF16), vmem((KLR, D), BF16), vmem((128 * G, D), BF16),
        vmem((D, D), BF16), vmem((D, D), BF16),
        vmem((G, S, 128), BF16), vmem((G, 128, S), BF16), vmem((H, VR, S), F32),
        vmem((D, S), F32),
        pltpu.SemaphoreType.DMA((10 + NB3,)), vmem((F,), BF16),
    ] + [vmem((S, BQ), F32)] * (2 * HPS) + [vmem((8, BQ), F32)] * (2 * HPS)
    out_t = pl.pallas_call(
        _kernel,
        out_shape=jax.ShapeDtypeStruct((D, S), BF16),
        in_specs=[hbm] * 6,
        out_specs=hbm,
        scratch_shapes=scratch,
        compiler_params=pltpu.CompilerParams(vmem_limit_bytes=120 * 1024 * 1024),
        name="fused_mha_mish",
    )(A_x.reshape(S, D).T, A_wqkv, A_wo, B_w1, B_b1, B_w2.T)
    return out_t.T.reshape(1, S, D)
```
